```python
import os as _os
_os.environ.setdefault("JAX_PLATFORMS", "cpu")
import jax
import jax.numpy as jnp

def _softmax(x, axis=-1):
    return jax.nn.softmax(x, axis=axis)
def _gelu(x):
    return jax.nn.gelu(x, approximate=True)
def _silu(x):
    return jax.nn.silu(x)
def _sigmoid(x):
    return jax.nn.sigmoid(x)
def _layernorm(x, axis=-1, eps=1e-5):
    m = jnp.mean(x, axis=axis, keepdims=True)
    v = jnp.var(x, axis=axis, keepdims=True)
    return (x - m) / jnp.sqrt(v + eps)
def _scatter_add(tgt, idx, src, axis=0):
    return tgt.at[idx].add(src)
def _segment_sum(src, seg, n):
    return jax.ops.segment_sum(src, seg, n)
class _Rng:
    def __init__(self, key):
        self._k = key
    def _next(self):
        self._k, sub = jax.random.split(self._k)
        return sub
    def normal(self, shape):
        return jax.random.normal(self._next(), shape, dtype=jnp.bfloat16)
    def randint(self, lo, hi, shape):
        return jax.random.randint(self._next(), shape, lo, hi, dtype=jnp.int32)
    def uniform(self, shape, lo=0.0, hi=1.0):
        return jax.random.uniform(self._next(), shape, jnp.bfloat16, lo, hi)
    def permutation(self, n):
        return jax.random.permutation(self._next(), n)


kernel_name = 'gated_mix__ssm_conv_s5__glu_gated_geglu__prompt'

def setup_inputs():
    _rng = _Rng(jax.random.key(int.from_bytes(__import__("os").urandom(4), "little")))
    _w = (lambda a: (lambda t: t.astype(jnp.bfloat16) if jnp.issubdtype(t.dtype, jnp.floating) else t)(jnp.asarray(a)))
    def _A_setup():
        B, S, D = 1, 2048, 448
        P = D
        Lambda_re = -0.5 * jnp.exp((lambda *s: _rng.normal(s) * 0.4)(P))
        Lambda_im = (lambda *s: _rng.normal(s) * 0.4)(P) * 1.0
        B_re = (lambda *s: _rng.normal(s) * 0.4)(P, D) * (D ** -0.5)
        B_im = (lambda *s: _rng.normal(s) * 0.4)(P, D) * (D ** -0.5)
        C_re = (lambda *s: _rng.normal(s) * 0.4)(D, P) * (P ** -0.5)
        C_im = (lambda *s: _rng.normal(s) * 0.4)(D, P) * (P ** -0.5)
        log_dt = (lambda *s: _rng.normal(s) * 0.4)(P) * 0.3 - 2.0
        Dskip = (lambda *s: _rng.normal(s) * 0.4)(D)
        return {
            "x": _w((lambda *s: _rng.normal(s) * 0.05)(B, S, D)),
            "Lambda_re": _w(Lambda_re),
            "Lambda_im": _w(Lambda_im),
            "B_re": _w(B_re),
            "B_im": _w(B_im),
            "C_re": _w(C_re),
            "C_im": _w(C_im),
            "log_dt": _w(log_dt),
            "Dskip": _w(Dskip),
        }
    _A_in = _A_setup()

    def _B_setup():
        B, S, Dm, Df = 1, 2048, 448, 1792
        return {
            "x": _w((lambda *s: _rng.normal(s) * 0.05)(B, S, Dm)),
            "w_gate": _w((lambda *s: _rng.normal(s) * 1.6)(Dm, Df) * (Dm ** -0.5)),
            "w_up": _w((lambda *s: _rng.normal(s) * 1.6)(Dm, Df) * (Dm ** -0.5)),
            "w_down": _w((lambda *s: _rng.normal(s) * 1.6)(Df, Dm) * (Df ** -0.5)),
        }
    _B_in = _B_setup()

    return {
        "A_x": _A_in["x"],
        "A_Lambda_re": _A_in["Lambda_re"],
        "A_Lambda_im": _A_in["Lambda_im"],
        "A_B_re": _A_in["B_re"],
        "A_B_im": _A_in["B_im"],
        "A_C_re": _A_in["C_re"],
        "A_C_im": _A_in["C_im"],
        "A_log_dt": _A_in["log_dt"],
        "A_Dskip": _A_in["Dskip"],
        "B_x": _B_in["x"],
        "B_w_gate": _B_in["w_gate"],
        "B_w_up": _B_in["w_up"],
        "B_w_down": _B_in["w_down"],
        "gate_w": _w((lambda *s: _rng.normal(s) * 0.05)(448) * 16.0),
    }

def reference(A_x, A_Lambda_re, A_Lambda_im, A_B_re, A_B_im, A_C_re, A_C_im, A_log_dt, A_Dskip, B_x, B_w_gate, B_w_up, B_w_down, gate_w):
    def _A_ref(x, Lambda_re, Lambda_im, B_re, B_im, C_re, C_im, log_dt, Dskip):
        Bsz, L, H = x.shape
        Lam = Lambda_re + 1j * Lambda_im
        Bmat = B_re + 1j * B_im
        Cmat = C_re + 1j * C_im
        dt = jnp.exp(log_dt)
        Lam_bar = jnp.exp(dt * Lam)
        B_bar = ((Lam_bar - 1.0) / Lam)[:, None] * Bmat
        Bu = jnp.einsum("bld,pd->blp", x + 0j, B_bar)
        h = jnp.zeros_like(Bu[:, 0, :])
        hs = []
        for t in range(L):
            h = Lam_bar[None, :] * h + Bu[:, t, :]
            hs.append(h)
        hseq = jnp.stack(hs, 1)
        y = 2.0 * jnp.einsum("blp,dp->bld", hseq, Cmat).real + x * Dskip[None, None, :]
        return y

    def _B_ref(x, w_gate, w_up, w_down):
        g = jnp.einsum("bsd,df->bsf", x, w_gate)
        u = jnp.einsum("bsd,df->bsf", x, w_up)
        h = _gelu(g) * u
        return jnp.einsum("bsf,fd->bsd", h, w_down)

    x = A_x
    g = _sigmoid((x * gate_w).sum(-1, keepdims=True))
    a = _A_ref(x, A_Lambda_re, A_Lambda_im, A_B_re, A_B_im, A_C_re, A_C_im, A_log_dt, A_Dskip)
    b = _B_ref(x, B_w_gate, B_w_up, B_w_down)
    return g * a + (1 - g) * b
```

```python
import functools
import numpy as np
import jax
import jax.numpy as jnp
from jax import lax
from jax.experimental import pallas as pl
from jax.experimental.pallas import tpu as pltpu

BF = jnp.bfloat16
F32 = jnp.float32
U32 = jnp.uint32
L = 2048
D = 448
FF = 1792
MB = 512
NB = L // MB
HB = MB // 2
TS = 65
KH = 256
DH = D // 2
NC = FF // 256


def _pk(v):
    return pltpu.bitcast(v, U32)


def _up(v):
    return pltpu.bitcast(v, BF)


def _nn(a, b):
    return jnp.dot(a, b, preferred_element_type=F32)


def _nt(a, b):
    return lax.dot_general(a, b, (((1,), (1,)), ((), ())), preferred_element_type=F32)


def _add(a, b):
    return (a.astype(F32) + b.astype(F32)).astype(BF)


def _sub(a, b):
    return (a.astype(F32) - b.astype(F32)).astype(BF)


def _comb(m):
    m1, m2, m3, m4, m5, m6, m7 = m
    return (m1 + m4 - m5 + m7, m3 + m5, m2 + m4, m1 - m2 + m3 + m6)


def _lhs_ops(a11, a12, a21, a22):
    return [_add(a11, a22), _add(a21, a22), a11, a22, _add(a11, a12), _sub(a21, a11), _sub(a12, a22)]


def _rhs_ops(b11, b12, b21, b22):
    return [_add(b11, b22), b11, _sub(b12, b22), _sub(b21, b11), b22, _add(b11, b12), _add(b21, b22)]


def _rhs_ops_f32(b11, b12, b21, b22):
    vals = [b11 + b22, b11, b12 - b22, b21 - b11, b22, b11 + b12, b21 + b22]
    return [v.astype(BF) for v in vals]


def _lhs_f32(a11, a12, a21, a22):
    return [a11 + a22, a21 + a22, a11, a22, a11 + a12, a21 - a11, a12 - a22]


def _rhs_f32(b11, b12, b21, b22):
    return [b11 + b22, b11, b12 - b22, b21 - b11, b22, b11 + b12, b21 + b22]


def _two_level(ops, blk):
    lvl1 = [[[None] * 2 for _ in range(2)] for _ in range(7)]
    for a in range(2):
        for v in range(2):
            o = ops(blk[a][v], blk[a][2 + v], blk[2 + a][v], blk[2 + a][2 + v])
            for i in range(7):
                lvl1[i][a][v] = o[i]
    lvl2 = [ops(g[0][0], g[0][1], g[1][0], g[1][1]) for g in lvl1]
    return lvl1, lvl2


ORDER = (3, 4, 6, 0, 2, 1, 5)


def _cmul(ar, ai, br, bi):
    return ar * br - ai * bi, ar * bi + ai * br


def _gelu_mul(g, u):
    return jax.nn.gelu(g, approximate=True) * u


def _zero_from(v):
    bits = pltpu.bitcast(v, U32)
    return (bits >> 31) >> 1


def _after(x, dep):
    z = _zero_from(dep)
    if x.dtype == U32:
        return x | z
    return pltpu.bitcast(pltpu.bitcast(x, U32) | z, F32)


def _delay(z, n):
    for _ in range(n):
        z = pltpu.roll(z, 1, 1)
    return z


def kernel(xt_hbm, lre_hbm, lim_hbm, bre_hbm, bim_hbm, cre_hbm, cim_hbm, ldt_hbm, dsk_hbm,
           wg_hbm, wu_hbm, wdt_hbm, gw_hbm,
           out_hbm,
           lre_v, lim_v, ldt_v, dsk_v, gw_v,
           xt_v, bre_v, bim_v, cre_v, cim_v, wg_v, wu_v, wdt_v,
           s_v, s2_v, xp_v, t1_v, tb_v, tb6_v, a2_v, ac_v,
           bu_v, hs_v, u2_v, uc_v, o_v, prm_v, col_v, carry_v, crow_v, g_v, yf_v,
           sem_small, sem_x, sem_b, sem_c, sem_w, sem_d, sem_o,
           *, cfg):
    R1 = cfg["R1"]
    NR = HB // R1
    small = [pltpu.make_async_copy(h, v, sem_small.at[i]) for i, (h, v) in enumerate(
        [(lre_hbm, lre_v), (lim_hbm, lim_v), (ldt_hbm, ldt_v), (dsk_hbm, dsk_v), (gw_hbm, gw_v)])]

    def xcp(b):
        return pltpu.make_async_copy(xt_hbm.at[:, pl.ds(b * MB, MB)], xt_v.at[:, pl.ds(b * MB, MB)], sem_x.at[b])

    def wcp(c, i):
        h, v = [(wg_hbm, wg_v), (wu_hbm, wu_v)][i]
        return pltpu.make_async_copy(h.at[:, pl.ds(c * 256, 256)], v.at[:, pl.ds(c * 256, 256)], sem_w.at[2 * c + i])

    dcp = pltpu.make_async_copy(wdt_hbm, wdt_v, sem_d.at[0])
    bcp = [pltpu.make_async_copy(bre_hbm, bre_v, sem_b.at[0]), pltpu.make_async_copy(bim_hbm, bim_v, sem_b.at[1])]
    ccp = [pltpu.make_async_copy(cre_hbm, cre_v, sem_c.at[0]), pltpu.make_async_copy(cim_hbm, cim_v, sem_c.at[1])]

    def start_loop(lo, hi, fn):
        def body(i, c):
            fn(i)
            return c
        lax.fori_loop(lo, hi, body, 0)

    def start_w(c):
        off = pl.multiple_of(c * 256, 256)
        for i, (h, v) in enumerate([(wg_hbm, wg_v), (wu_hbm, wu_v)]):
            pltpu.make_async_copy(h.at[:, pl.ds(off, 256)], v.at[:, pl.ds(off, 256)], sem_w.at[2 * c + i]).start()

    def start_x(b):
        off = pl.multiple_of(b * MB, MB)
        pltpu.make_async_copy(xt_hbm.at[:, pl.ds(off, MB)], xt_v.at[:, pl.ds(off, MB)], sem_x.at[b]).start()

    def start_rest(k):
        @pl.when(k == 0)
        def _():
            dcp.start()

        @pl.when(k == 1)
        def _():
            for c in bcp:
                c.start()

        @pl.when(k == 2)
        def _():
            for c in ccp:
                c.start()

    xcp(0).start()
    for c in small:
        c.start()
    start_loop(0, NC, start_w)
    start_loop(0, 3, start_rest)
    start_loop(1, NB, start_x)

    bu_v[:, MB:MB + 8, :] = jnp.zeros((8, 8, 128), F32)

    def params():
        lre = lre_v[...].astype(F32)[None, :]
        lim = lim_v[...].astype(F32)[None, :]
        dt = jnp.exp(ldt_v[...].astype(F32)[None, :]).astype(BF).astype(F32)
        ea = jnp.exp(dt * lre)
        lbr = ea * jnp.cos(dt * lim)
        lbi = ea * jnp.sin(dt * lim)
        den = lre * lre + lim * lim
        nr = lbr - 1.0
        crow_v[0:1, :] = (nr * lre + lbi * lim) / den
        crow_v[1:2, :] = (lbi * lre - nr * lim) / den
        pr, pi = lbr, lbi
        for _ in range(6):
            pr, pi = pr * pr - pi * pi, 2.0 * pr * pi
        p1r, p1i = _cmul(pr, pi, lbr, lbi)
        p2r, p2i = p1r * p1r - p1i * p1i, 2.0 * p1r * p1i
        p4r, p4i = p2r * p2r - p2i * p2i, 2.0 * p2r * p2i

        def tiles4(vr, vi):
            out = []
            for j in range(3):
                out.append((vr[:, 128 * j:128 * (j + 1)], vi[:, 128 * j:128 * (j + 1)]))
            hr, hi = vr[:, 384:448], vi[:, 384:448]
            out.append((jnp.concatenate([hr, hr], axis=1), jnp.concatenate([hi, -hi], axis=1)))
            return out

        for k, (vr, vi) in enumerate([(lbr, lbi), (p1r, p1i), (p2r, p2i), (p4r, p4i)]):
            for j, (tr, ti) in enumerate(tiles4(vr, vi)):
                prm_v[8 * k + 2 * j:8 * k + 2 * j + 1, :] = tr
                prm_v[8 * k + 2 * j + 1:8 * k + 2 * j + 2, :] = ti
        col_v[0] = jnp.broadcast_to(dsk_v[...].astype(F32)[None, :], (128, D)).T
        col_v[1] = jnp.broadcast_to(gw_v[...].astype(F32)[None, :], (128, D)).T
        carry_v[...] = jnp.zeros((8, 128), F32)

    def prm(k, j, im):
        r = 8 * k + 2 * j + im
        return jnp.broadcast_to(prm_v[r:r + 1, :], (8, 128))

    def prep_x(b):
        zrow = jnp.zeros((2 * KH - D, 128), BF)
        xs = []
        for tt in range(4):
            xt = xt_v[:, b * MB + 128 * tt:b * MB + 128 * (tt + 1)]
            x = jnp.concatenate([xt, zrow], axis=0).T
            xp_v[64 * tt:64 * (tt + 1), :] = _pk(x)
            xs.append(x)
        blk = [[xs[r][:, 128 * k:128 * (k + 1)].astype(F32) for k in range(4)] for r in range(4)]
        lvl1, lvl2 = _two_level(_lhs_f32, blk)
        for i in range(7):
            for a in range(2):
                if i in (2, 3):
                    o = xs[(0 if i == 2 else 2) + a][:, (0 if i == 2 else KH):(KH if i == 2 else 2 * KH)]
                else:
                    o = jnp.concatenate([lvl1[i][a][0], lvl1[i][a][1]], axis=1).astype(BF)
                s_v[i * 128 + 64 * a:i * 128 + 64 * (a + 1), :] = _pk(o)
            for j in range(7):
                n = 7 * i + j
                s2_v[(n // 2) * 64:(n // 2 + 1) * 64, (n % 2) * 128:(n % 2 + 1) * 128] = _pk(lvl2[i][j].astype(BF))

    def prep_b():
        zpad = jnp.zeros((128, 2 * KH - D), BF)

        def k2(ref, r0, n):
            return jnp.concatenate([ref[r0:r0 + n, KH:D], zpad[0:n]], axis=1)
        for j in range(3):
            r0 = 128 * j
            ops = _rhs_ops(bre_v[r0:r0 + 128, 0:KH], bim_v[r0:r0 + 128, 0:KH], k2(bre_v, r0, 128), k2(bim_v, r0, 128))
            for i, o in enumerate(ops):
                tb_v[i * 192 + r0 // 2:i * 192 + r0 // 2 + 64, :] = _pk(o)
        tb6_v[0:32, 0:KH] = _pk(bre_v[384:448, 0:KH])
        tb6_v[32:64, 0:KH] = _pk(bim_v[384:448, 0:KH])
        tb6_v[0:32, KH:2 * KH] = _pk(k2(bre_v, 384, 64))
        tb6_v[32:64, KH:2 * KH] = _pk(k2(bim_v, 384, 64))

    def prep_w1(c):
        zpad = jnp.zeros((2 * KH - D, 128), F32)
        blk = [[None] * 4 for _ in range(4)]
        for q, ref in enumerate((wg_v, wu_v)):
            w = ref[:, 256 * c:256 * (c + 1)].astype(F32)
            for nu in range(2):
                for k in range(4):
                    if k < 3:
                        blk[k][2 * q + nu] = w[128 * k:128 * (k + 1), 128 * nu:128 * (nu + 1)]
                    else:
                        blk[k][2 * q + nu] = jnp.concatenate([w[384:448, 128 * nu:128 * (nu + 1)], zpad], axis=0)
        _, lvl2 = _two_level(_rhs_f32, blk)
        for i in range(7):
            for j in range(7):
                n = 7 * i + j
                t1_v[n * 64:(n + 1) * 64, 128 * c:128 * (c + 1)] = _pk(lvl2[i][j].astype(BF))

    def prep_w2():
        for c in range(NC):
            e = slice(256 * c, 256 * c + 128)
            o = slice(256 * c + 128, 256 * c + 256)
            ops = _lhs_ops(wdt_v[0:DH, e], wdt_v[0:DH, o], wdt_v[DH:D, e], wdt_v[DH:D, o])
            for i, v in enumerate(ops):
                a2_v[i * 112:(i + 1) * 112, 128 * c:128 * (c + 1)] = _pk(v)

    def prep_c():
        cr = 2.0 * crow_v[0:1, :]
        ci = 2.0 * crow_v[1:2, :]
        parts = []
        for hf in range(2):
            rs = slice(DH * hf, DH * (hf + 1))
            cre = cre_v[rs, :].astype(F32)
            cim = cim_v[rs, :].astype(F32)
            are = cre * cr - cim * ci
            aim = -(cre * ci + cim * cr)
            ac_v[112 * hf:112 * (hf + 1), 384:512] = _pk(
                jnp.concatenate([are[:, 384:448], aim[:, 384:448]], axis=1).astype(BF))
            parts.append((are, aim))
        for j in range(3):
            cs = slice(128 * j, 128 * (j + 1))
            ops = _lhs_f32(parts[0][0][:, cs], parts[0][1][:, cs], parts[1][0][:, cs], parts[1][1][:, cs])
            for i, v in enumerate(ops):
                ac_v[i * 112:(i + 1) * 112, cs] = _pk(v.astype(BF))

    def s_raw(i, rs):
        return s_v[i * 128 + rs.start // 2:i * 128 + rs.stop // 2, :]

    def s_op(i, rs):
        return _up(s_raw(i, rs))

    def ssm_s1(b, rr, j):
        rs = slice(rr * R1, (rr + 1) * R1)
        m = [None] * 7
        for i in cfg["ord_s1"]:
            m[i] = _nt(s_op(i, rs), _up(tb_v[i * 192 + 64 * j:i * 192 + 64 * (j + 1), :]))
        c11, c12, c21, c22 = _comb(m)
        bu_v[2 * j, rr * R1:(rr + 1) * R1, :] = c11
        bu_v[2 * j + 1, rr * R1:(rr + 1) * R1, :] = c12
        bu_v[2 * j, HB + rr * R1:HB + (rr + 1) * R1, :] = c21
        bu_v[2 * j + 1, HB + rr * R1:HB + (rr + 1) * R1, :] = c22

    def ssm_s16(b, tt):
        r0 = 64 * tt
        z = _nt(_up(xp_v[r0:r0 + 64, :]), _up(tb6_v[...]))
        bu_v[6, 128 * tt:128 * (tt + 1), :] = z
        bu_v[7, 128 * tt:128 * (tt + 1), :] = pltpu.roll(z, 64, 1)

    def gated(raw, z):
        if z is None:
            return raw
        top = jnp.concatenate([raw[0:8, 0:128] | z, raw[0:8, 128:]], axis=1)
        return jnp.concatenate([top, raw[8:, :]], axis=0)

    def ffn_s1(b, c, rr, R1=R1, z=None):
        r0 = rr * R1 // 2
        outer = [None] * 7
        for i in ORDER:
            p = [None] * 7
            for j in ORDER:
                n = 7 * i + j
                lhs = s2_v[(n // 2) * 64 + r0:(n // 2) * 64 + r0 + R1 // 2, (n % 2) * 128:(n % 2 + 1) * 128]
                p[j] = _nn(_up(lhs), _up(t1_v[n * 64:(n + 1) * 64, 128 * c:128 * (c + 1)]))
            outer[i] = _comb(p)
        hh = {}
        for a in range(2):
            for nu in range(2):
                g1, u1, g2, u2 = _comb([outer[i][2 * a + nu] for i in range(7)])
                hh[(0, a, nu)] = _gelu_mul(g1, u1)
                hh[(1, a, nu)] = _gelu_mul(g2, u2)
        for a in range(2):
            ops = _rhs_ops_f32(hh[(0, a, 0)], hh[(1, a, 0)], hh[(0, a, 1)], hh[(1, a, 1)])
            for i, o in enumerate(ops):
                u2_v[i * 128 + 64 * a + r0:i * 128 + 64 * a + r0 + R1 // 2, 128 * c:128 * (c + 1)] = _pk(o)

    def ffn_s2(q, i):
        return _nt(_up(a2_v[i * 112:(i + 1) * 112, :]), _up(u2_v[i * 128 + 64 * q:i * 128 + 64 * (q + 1), :]))

    def ssm_s2(q, i):
        return _nt(_up(ac_v[i * 112:(i + 1) * 112, 0:384]), _up(uc_v[i * 128 + 64 * q:i * 128 + 64 * (q + 1), 0:384]))

    def ssm_p6(tt):
        return _nt(_up(ac_v[0:224, 384:512]), _up(uc_v[64 * tt:64 * (tt + 1), 384:512]))

    def scan():
        groups = cfg["scan_groups"]
        zero = jnp.zeros((8, 128), F32)
        er, ei = {}, {}
        dep = None
        for grp in groups:
            for j in grp:
                er[j] = zero if dep is None else _after(zero, dep)
                ei[j] = er[j]
            lr = {j: prm(0, j, 0) for j in grp}
            li = {j: prm(0, j, 1) for j in grp}
            for t in range(TS):
                for j in grp:
                    br = bu_v[2 * j, pl.ds(t, 8, stride=TS), :]
                    bi = bu_v[2 * j + 1, pl.ds(t, 8, stride=TS), :]
                    er[j], ei[j] = lr[j] * er[j] - li[j] * ei[j] + br, lr[j] * ei[j] + li[j] * er[j] + bi
            if cfg["scan_chain"]:
                dep = ei[grp[-1]]
        row = lax.broadcasted_iota(jnp.int32, (8, 128), 0)
        sr, si = {}, {}
        for j in range(4):
            cin_r = jnp.broadcast_to(carry_v[2 * j:2 * j + 1, :], (8, 128))
            cin_i = jnp.broadcast_to(carry_v[2 * j + 1:2 * j + 2, :], (8, 128))
            xr = jnp.where(row == 0, cin_r, pltpu.roll(er[j], 1, 0))
            xi = jnp.where(row == 0, cin_i, pltpu.roll(ei[j], 1, 0))
            for k, sh in enumerate([1, 2, 4]):
                ar, ai = prm(1 + k, j, 0), prm(1 + k, j, 1)
                yr = jnp.where(row >= sh, pltpu.roll(xr, sh, 0), 0.0)
                yi = jnp.where(row >= sh, pltpu.roll(xi, sh, 0), 0.0)
                xr, xi = xr + (ar * yr - ai * yi), xi + (ar * yi + ai * yr)
            sr[j], si[j] = xr, xi
        for gi, grp in enumerate(groups):
            if cfg["scan_chain"]:
                for j in grp:
                    sr[j] = _after(sr[j], dep)
            lr = {j: prm(0, j, 0) for j in grp}
            li = {j: prm(0, j, 1) for j in grp}
            for t in range(TS):
                for j in grp:
                    br = bu_v[2 * j, pl.ds(t, 8, stride=TS), :]
                    bi = bu_v[2 * j + 1, pl.ds(t, 8, stride=TS), :]
                    sr[j], si[j] = lr[j] * sr[j] - li[j] * si[j] + br, lr[j] * si[j] + li[j] * sr[j] + bi
                    if j < 3:
                        hs_v[2 * j, pl.ds(t, 8, stride=TS), :] = sr[j]
                        hs_v[2 * j + 1, pl.ds(t, 8, stride=TS), :] = si[j]
                    else:
                        hs_v[6, pl.ds(t, 8, stride=TS), :] = sr[j]
                    if t == MB - 1 - 7 * TS:
                        carry_v[2 * j:2 * j + 1, :] = sr[j][7:8, :]
                        carry_v[2 * j + 1:2 * j + 2, :] = si[j][7:8, :]
            dep = sr[grp[-1]]

    def h_ops():
        for q in range(2):
            m1 = slice(128 * q, 128 * (q + 1))
            m2 = slice(HB + 128 * q, HB + 128 * (q + 1))
            for j in range(3):
                ops = _rhs_ops_f32(hs_v[2 * j, m1, :], hs_v[2 * j, m2, :], hs_v[2 * j + 1, m1, :], hs_v[2 * j + 1, m2, :])
                for i, o in enumerate(ops):
                    uc_v[i * 128 + 64 * q:i * 128 + 64 * (q + 1), 128 * j:128 * (j + 1)] = _pk(o)
        for tt in range(4):
            uc_v[64 * tt:64 * (tt + 1), 384:512] = _pk(hs_v[6, 128 * tt:128 * (tt + 1), :].astype(BF))

    def gates(b):
        for tt in range(4):
            xt = xt_v[:, b * MB + 128 * tt:b * MB + 128 * (tt + 1)].astype(F32)
            z = jnp.sum(xt * col_v[1], axis=0, keepdims=True)
            g_v[tt:tt + 1, :] = jax.nn.sigmoid(z)

    def epilogue(b, tt, dh, ys):
        rs = slice(DH * dh, DH * (dh + 1))
        ts = slice(128 * tt, 128 * (tt + 1))
        xt = xt_v[rs, b * MB + 128 * tt:b * MB + 128 * (tt + 1)].astype(F32)
        g = g_v[tt:tt + 1, :]
        a = ys + xt * col_v[0, rs, :]
        o_v[b, rs, ts] = g * a + (1.0 - g) * yf_v[rs, ts]
        cp = pltpu.make_async_copy(o_v.at[b, rs, ts], out_hbm.at[rs, b * MB + 128 * tt:b * MB + 128 * (tt + 1)],
                                   sem_o.at[b * 8 + 2 * tt + dh])
        cp.start()
        return cp

    out_cps = []

    def stage1_ssm(b):
        for rr in range(NR):
            for j in range(3):
                ssm_s1(b, rr, j)
        for tt in range(4):
            ssm_s16(b, tt)

    def stage1_ffn(b, chunks, halves=(0, 1), gates_=None):
        r1 = cfg["RF"]
        n = 128 // r1
        for c in chunks:
            for rr in range(n):
                if (2 * rr) // n in halves:
                    ffn_s1(b, c, rr, r1, (gates_ or {}).get((c, rr)))

    def pull(v, n=None):
        n = cfg["delay"] if n is None else n
        return _delay(_zero_from(v) if v.dtype != U32 else (v >> 31) >> 1, n)

    def t1_tok(c):
        return None

    def stage2_ffn(b):
        for q in range(2):
            f = [None] * 7
            for i in cfg["ord_f2"]:
                f[i] = ffn_s2(q, i)
            c11, c12, c21, c22 = _comb(f)
            yf_v[0:DH, 128 * q:128 * (q + 1)] = c11
            yf_v[0:DH, HB + 128 * q:HB + 128 * (q + 1)] = c12
            yf_v[DH:D, 128 * q:128 * (q + 1)] = c21
            yf_v[DH:D, HB + 128 * q:HB + 128 * (q + 1)] = c22

    def stage2_ssm(b):
        for q in range(2):
            t1, t2 = q, 2 + q
            p6a = ssm_p6(t1)
            p6b = ssm_p6(t2)
            ms = [None] * 7
            for i in cfg["ord_s2"]:
                ms[i] = ssm_s2(q, i)
            s11, s12, s21, s22 = _comb(ms)
            out_cps.append(epilogue(b, t2, 0, s12 + p6b[0:DH]))
            out_cps.append(epilogue(b, t1, 1, s21 + p6a[DH:D]))
            out_cps.append(epilogue(b, t2, 1, s22 + p6b[DH:D]))
            out_cps.append(epilogue(b, t1, 0, s11 + p6a[0:DH]))

    def wait_w(cs):
        for c in cs:
            wcp(c, 0).wait()
            wcp(c, 1).wait()

    xcp(0).wait()
    wait_w([0])
    for c in small:
        c.wait()
    prep_x(0)
    prep_w1(0)
    stage1_ffn(0, [0])
    wait_w([1, 2])
    for c in (1, 2):
        prep_w1(c)
        stage1_ffn(0, [c])
    params()
    wait_w([3, 4, 5, 6])
    for c in (3, 4, 5, 6):
        prep_w1(c)
        stage1_ffn(0, [c])
    dcp.wait()
    for c in bcp:
        c.wait()
    prep_b()
    for b in range(NB):
        if b > 0:
            stage1_ffn(b, range(NC))
        stage1_ssm(b)
        if b == 0:
            for c in ccp:
                c.wait()
            for bb in range(1, NB):
                xcp(bb).wait()
            prep_w2()
            prep_c()
        stage2_ffn(b)
        scan()
        h_ops()
        gates(b)
        if b + 1 < NB:
            prep_x(b + 1)
        stage2_ssm(b)
    for cp in out_cps:
        cp.wait()


_CFG = dict(RF=64, ord_s1=ORDER, ord_f2=ORDER, ord_s2=ORDER, delay=3, pull=True, grr=3, R1=64, R1_0=64,
            scan_groups=[[0], [1], [2], [3]], scan_chain=True)


@jax.jit
def pallas_gated_mix__ssm_conv_s5__glu_gated_geglu__prompt_kernel(
    A_x: jax.Array,
    A_Lambda_re: jax.Array,
    A_Lambda_im: jax.Array,
    A_B_re: jax.Array,
    A_B_im: jax.Array,
    A_C_re: jax.Array,
    A_C_im: jax.Array,
    A_log_dt: jax.Array,
    A_Dskip: jax.Array,
    B_x: jax.Array,
    B_w_gate: jax.Array,
    B_w_up: jax.Array,
    B_w_down: jax.Array,
    gate_w: jax.Array,
):
    xt = A_x.reshape(L, D).T
    wdt = B_w_down.T
    any_spec = pl.BlockSpec(memory_space=pl.ANY)
    V = pltpu.VMEM
    scratch = [V((D,), BF)] * 5 + [
        V((D, L), BF), V((D, D), BF), V((D, D), BF), V((D, D), BF), V((D, D), BF),
        V((D, FF), BF), V((D, FF), BF), V((D, FF), BF),
        V((7 * 128, KH), U32),
        V((25 * 64, 256), U32),
        V((MB // 2, 2 * KH), U32),
        V((49 * 64, FF // 2), U32),
        V((7 * 192, KH), U32),
        V((64, 2 * KH), U32),
        V((7 * DH // 2, FF // 2), U32),
        V((7 * DH // 2, 512), U32),
        V((8, MB + 8, 128), F32),
        V((7, MB + 8, 128), F32),
        V((7 * HB // 2, FF // 2), U32),
        V((7 * HB // 2, 512), U32),
        V((NB, D, MB), F32),
        V((32, 128), F32),
        V((2, D, 128), F32),
        V((8, 128), F32),
        V((8, D), F32),
        V((8, 128), F32),
        V((D, MB), F32),
    ] + [pltpu.SemaphoreType.DMA((n,)) for n in (5, NB, 2, 2, 14, 1, 32)]
    out = pl.pallas_call(
        functools.partial(kernel, cfg=_CFG),
        out_shape=jax.ShapeDtypeStruct((D, L), F32),
        in_specs=[any_spec] * 13,
        out_specs=any_spec,
        scratch_shapes=scratch,
        compiler_params=pltpu.CompilerParams(vmem_limit_bytes=110 * 1024 * 1024),
        name="gmix",
    )(xt, A_Lambda_re, A_Lambda_im, A_B_re, A_B_im, A_C_re, A_C_im, A_log_dt, A_Dskip, B_w_gate, B_w_up, wdt, gate_w)
    return out.T.reshape(1, L, D)
```

```python
import functools

import numpy as np
import jax
import jax.numpy as jnp
from jax import lax
import jax.experimental.pallas as pl
import jax.experimental.pallas.tpu as pltpu

BF = jnp.bfloat16
F32 = jnp.float32
U32 = jnp.uint32

L = 2048
D = 448
FF = 1792
MB = 512
NB = L // MB
HB = MB // 2
DH = D // 2
KH = 256
NC = FF // 256
TS = 65
RF = 64
R1 = 64
ORDER = (3, 4, 6, 0, 2, 1, 5)
ORDER_OUT = (2, 4, 1, 3, 0, 5, 6)
_C1 = float(np.sqrt(2.0 / np.pi))
_C2 = float(np.sqrt(2.0 / np.pi) * 0.044715)


def _pk(v):
    return pltpu.bitcast(v, U32)


def _up(v):
    return pltpu.bitcast(v, BF)


def _nn(a, b):
    return jnp.dot(a, b, preferred_element_type=F32)


def _nt(a, b):
    return lax.dot_general(a, b, (((1,), (1,)), ((), ())), preferred_element_type=F32)


def _lhs(a11, a12, a21, a22):
    return [a11 + a22, a21 + a22, a11, a22, a11 + a12, a21 - a11, a12 - a22]


def _rhs(b11, b12, b21, b22):
    return [b11 + b22, b11, b12 - b22, b21 - b11, b22, b11 + b12, b21 + b22]


def _comb(m):
    m1, m2, m3, m4, m5, m6, m7 = m
    return (m1 + m4 - m5 + m7, m3 + m5, m2 + m4, m1 - m2 + m3 + m6)


def _one_level(ops, a, b, c, d):
    raw = (a, b, c, d)
    out = []
    for v in ops(*[x.astype(F32) for x in raw]):
        out.append(v.astype(BF))
    plain = {2: 0, 3: 3} if ops is _lhs else {1: 0, 4: 3}
    for i, k in plain.items():
        out[i] = raw[k]
    return out


def _two_level(ops, blk):
    lvl1 = []
    for i in range(7):
        lvl1.append([[None, None], [None, None]])
    for a in range(2):
        for v in range(2):
            o = ops(blk[a][v], blk[a][2 + v], blk[2 + a][v], blk[2 + a][2 + v])
            for i in range(7):
                lvl1[i][a][v] = o[i]
    return lvl1, [ops(g[0][0], g[0][1], g[1][0], g[1][1]) for g in lvl1]


def _gelu_mul2(g, u):
    return (g * u) * (1.0 + jnp.tanh(g * (_C1 + _C2 * (g * g))))


def _after(x, dep):
    z = (pltpu.bitcast(dep, U32) >> 31) >> 1
    return pltpu.bitcast(pltpu.bitcast(x, U32) | z, F32)


def _kernel(xt_hbm, lre_hbm, lim_hbm, bre_hbm, bim_hbm, cre_hbm, cim_hbm, ldt_hbm, dsk_hbm,
            wg_hbm, wu_hbm, wdt_hbm, gw_hbm,
            out_hbm,
            lre_v, lim_v, ldt_v, dsk_v, gw_v,
            xt_v, bre_v, bim_v, cre_v, cim_v, wg_v, wu_v, wdt_v,
            s1_v, s2_v, xp_v, t2_v, tb2_v, tb1_v, tb6_v, a2_v, ac_v, u2_v, uc_v,
            bu_v, hs_v, yf_v, o_v, prm_v, col_v, carry_v, crow_v, g_v,
            sem_small, sem_x, sem_b, sem_c, sem_w, sem_d, sem_o):
    small = [pltpu.make_async_copy(h, v, sem_small.at[i]) for i, (h, v) in enumerate(
        [(lre_hbm, lre_v), (lim_hbm, lim_v), (ldt_hbm, ldt_v), (dsk_hbm, dsk_v), (gw_hbm, gw_v)])]
    dcp = pltpu.make_async_copy(wdt_hbm, wdt_v, sem_d.at[0])
    bcp = [pltpu.make_async_copy(bre_hbm, bre_v, sem_b.at[0]), pltpu.make_async_copy(bim_hbm, bim_v, sem_b.at[1])]
    ccp = [pltpu.make_async_copy(cre_hbm, cre_v, sem_c.at[0]), pltpu.make_async_copy(cim_hbm, cim_v, sem_c.at[1])]

    def cols(start, size):
        if isinstance(start, int):
            return slice(start, start + size)
        return pl.ds(pl.multiple_of(start, 128), size)

    def xcp(b):
        return pltpu.make_async_copy(xt_hbm.at[:, cols(b * MB, MB)], xt_v.at[:, cols(b * MB, MB)], sem_x.at[b])

    def wcp(c):
        return [pltpu.make_async_copy(h.at[:, cols(c * 256, 256)], v.at[:, cols(c * 256, 256)], sem_w.at[2 * c + i])
                for i, (h, v) in enumerate([(wg_hbm, wg_v), (wu_hbm, wu_v)])]

    def ocp(b, tt, dh):
        rs = slice(DH * dh, DH * (dh + 1))
        return pltpu.make_async_copy(o_v.at[b, rs, 128 * tt:128 * (tt + 1)],
                                     out_hbm.at[rs, cols(b * MB + 128 * tt, 128)], sem_o.at[b * 8 + 2 * tt + dh])

    def start_in_order(lo, hi, fn):
        def body(i, c):
            fn(i)
            return c
        lax.fori_loop(lo, hi, body, 0)

    def start_w(c):
        for cp in wcp(c):
            cp.start()

    def start_rest(k):
        for n, group in enumerate([[dcp], bcp, ccp]):
            @pl.when(k == n)
            def _():
                for cp in group:
                    cp.start()

    xcp(0).start()
    for cp in small:
        cp.start()
    start_in_order(0, NC, start_w)
    start_in_order(0, 3, start_rest)
    start_in_order(1, NB, lambda b: xcp(b).start())

    bu_v[:, MB:MB + 8, :] = jnp.zeros((8, 8, 128), F32)

    def params():
        lre = lre_v[...].astype(F32)[None, :]
        lim = lim_v[...].astype(F32)[None, :]
        dt = jnp.exp(ldt_v[...].astype(F32)[None, :]).astype(BF).astype(F32)
        ea = jnp.exp(dt * lre)
        lbr = ea * jnp.cos(dt * lim)
        lbi = ea * jnp.sin(dt * lim)
        den = lre * lre + lim * lim
        nr = lbr - 1.0
        crow_v[0:1, :] = (nr * lre + lbi * lim) / den
        crow_v[1:2, :] = (lbi * lre - nr * lim) / den
        pr, pi = lbr, lbi
        for _ in range(6):
            pr, pi = pr * pr - pi * pi, 2.0 * pr * pi
        p1r, p1i = pr * lbr - pi * lbi, pr * lbi + pi * lbr
        p2r, p2i = p1r * p1r - p1i * p1i, 2.0 * p1r * p1i
        p4r, p4i = p2r * p2r - p2i * p2i, 2.0 * p2r * p2i
        for k, (vr, vi) in enumerate([(lbr, lbi), (p1r, p1i), (p2r, p2i), (p4r, p4i)]):
            for j in range(4):
                if j < 3:
                    tr, ti = vr[:, 128 * j:128 * (j + 1)], vi[:, 128 * j:128 * (j + 1)]
                else:
                    hr, hi = vr[:, 384:448], vi[:, 384:448]
                    tr, ti = jnp.concatenate([hr, hr], axis=1), jnp.concatenate([hi, -hi], axis=1)
                prm_v[8 * k + 2 * j:8 * k + 2 * j + 1, :] = tr
                prm_v[8 * k + 2 * j + 1:8 * k + 2 * j + 2, :] = ti
        col_v[0] = jnp.broadcast_to(dsk_v[...].astype(F32)[None, :], (128, D)).T
        col_v[1] = jnp.broadcast_to(gw_v[...].astype(F32)[None, :], (128, D)).T
        carry_v[...] = jnp.zeros((8, 128), F32)

    def prm(k, j, im):
        r = 8 * k + 2 * j + im
        return jnp.broadcast_to(prm_v[r:r + 1, :], (8, 128))

    def slot2(n):
        return (n // 2) * 64, slice((n % 2) * 128, (n % 2 + 1) * 128)

    def prep_x(b):
        zrow = jnp.zeros((2 * KH - D, 128), BF)
        xs = []
        for tt in range(4):
            x = jnp.concatenate([xt_v[:, cols(b * MB + 128 * tt, 128)], zrow], axis=0).T
            xp_v[64 * tt:64 * (tt + 1), :] = _pk(x)
            xs.append(x)
        lvl1, lvl2 = _two_level(_lhs, [[xs[r][:, 128 * k:128 * (k + 1)].astype(F32) for k in range(4)]
                                       for r in range(4)])
        for i in range(7):
            for a in range(2):
                if i == 2:
                    o = xs[a][:, 0:KH]
                elif i == 3:
                    o = xs[2 + a][:, KH:2 * KH]
                else:
                    o = jnp.concatenate(lvl1[i][a], axis=1).astype(BF)
                s1_v[i * 128 + 64 * a:i * 128 + 64 * (a + 1), :] = _pk(o)
            for j in range(7):
                r, lanes = slot2(7 * i + j)
                s2_v[r:r + 64, lanes] = _pk(lvl2[i][j].astype(BF))

    def prep_w1(c):
        zpad = jnp.zeros((2 * KH - D, 128), F32)
        blk = [[None] * 4 for _ in range(4)]
        for q, ref in enumerate((wg_v, wu_v)):
            w = ref[:, 256 * c:256 * (c + 1)].astype(F32)
            for nu in range(2):
                for k in range(4):
                    t = w[128 * k:min(128 * (k + 1), D), 128 * nu:128 * (nu + 1)]
                    blk[k][2 * q + nu] = t if k < 3 else jnp.concatenate([t, zpad], axis=0)
        _, lvl2 = _two_level(_rhs, blk)
        for n in range(49):
            t2_v[n * 64:(n + 1) * 64, 128 * c:128 * (c + 1)] = _pk(lvl2[n // 7][n % 7].astype(BF))

    def prep_b():
        zpad = jnp.zeros((128, 2 * KH - D), BF)

        def k2(ref, r0, n):
            return jnp.concatenate([ref[r0:r0 + n, KH:D], zpad[0:n]], axis=1)
        blk = [[None] * 4 for _ in range(4)]
        for q, ref in enumerate((bre_v, bim_v)):
            for nu in range(2):
                w = jnp.concatenate([ref[128 * nu:128 * (nu + 1), :].astype(F32), zpad.astype(F32)], axis=1)
                for k in range(4):
                    blk[k][2 * q + nu] = w[:, 128 * k:128 * (k + 1)]
        _, lvl2 = _two_level(_rhs, blk)
        for n in range(49):
            r, lanes = slot2(n)
            tb2_v[r:r + 64, lanes] = _pk(lvl2[n // 7][n % 7].astype(BF))
        ops = _one_level(_rhs, bre_v[256:384, 0:KH], bim_v[256:384, 0:KH], k2(bre_v, 256, 128), k2(bim_v, 256, 128))
        for i, o in enumerate(ops):
            tb1_v[i * 64:(i + 1) * 64, :] = _pk(o)
        tb6_v[0:32, 0:KH] = _pk(bre_v[384:448, 0:KH])
        tb6_v[32:64, 0:KH] = _pk(bim_v[384:448, 0:KH])
        tb6_v[0:32, KH:2 * KH] = _pk(k2(bre_v, 384, 64))
        tb6_v[32:64, KH:2 * KH] = _pk(k2(bim_v, 384, 64))

    def prep_w2():
        for c in range(NC):
            e = slice(256 * c, 256 * c + 128)
            o = slice(256 * c + 128, 256 * c + 256)
            ops = _one_level(_lhs, wdt_v[0:DH, e], wdt_v[0:DH, o], wdt_v[DH:D, e], wdt_v[DH:D, o])
            for i, v in enumerate(ops):
                a2_v[i * 112:(i + 1) * 112, 128 * c:128 * (c + 1)] = _pk(v)

    def prep_c():
        cr = 2.0 * crow_v[0:1, :]
        ci = 2.0 * crow_v[1:2, :]
        parts = []
        for hf in range(2):
            cre = cre_v[DH * hf:DH * (hf + 1), :].astype(F32)
            cim = cim_v[DH * hf:DH * (hf + 1), :].astype(F32)
            are = cre * cr - cim * ci
            aim = -(cre * ci + cim * cr)
            ac_v[112 * hf:112 * (hf + 1), 384:512] = _pk(
                jnp.concatenate([are[:, 384:448], aim[:, 384:448]], axis=1).astype(BF))
            parts.append((are, aim))
        for j in range(3):
            cs = slice(128 * j, 128 * (j + 1))
            ops = _lhs(parts[0][0][:, cs], parts[0][1][:, cs], parts[1][0][:, cs], parts[1][1][:, cs])
            for i, v in enumerate(ops):
                ac_v[i * 112:(i + 1) * 112, cs] = _pk(v.astype(BF))

    def two_level_products(r0, rows, dot, rhs):
        outer = [None] * 7
        for i in ORDER:
            p = [None] * 7
            for j in ORDER:
                r, lanes = slot2(7 * i + j)
                p[j] = dot(_up(s2_v[r + r0 // 2:r + (r0 + rows) // 2, lanes]), _up(rhs(7 * i + j)))
            outer[i] = _comb(p)
        out = {}
        for a in range(2):
            for nu in range(2):
                c = _comb([outer[i][2 * a + nu] for i in range(7)])
                for p in range(2):
                    for q in range(2):
                        out[(2 * p + a, q, nu)] = c[2 * p + q]
        return out

    def ffn_stage1(chunks):
        for c in chunks:
            for rr in range(128 // RF):
                z = two_level_products(rr * RF, RF, _nn, lambda n: t2_v[n * 64:(n + 1) * 64, 128 * c:128 * (c + 1)])
                hh = {(tt, nu): _gelu_mul2(z[(tt, 0, nu)], z[(tt, 1, nu)]) for tt in range(4) for nu in range(2)}
                for a in range(2):
                    ops = _rhs(hh[(a, 0)], hh[(2 + a, 0)], hh[(a, 1)], hh[(2 + a, 1)])
                    for i, o in enumerate(ops):
                        r = i * 128 + 64 * a + rr * RF // 2
                        u2_v[r:r + RF // 2, 128 * c:128 * (c + 1)] = _pk(o.astype(BF))

    def ssm_stage1():
        def rhs(n):
            r, lanes = slot2(n)
            return tb2_v[r:r + 64, lanes]
        z = two_level_products(0, 128, _nt, rhs)
        for (tt, q, nu), v in z.items():
            bu_v[2 * nu + q, 128 * tt:128 * (tt + 1), :] = v
        for rr in range(HB // R1):
            m = [None] * 7
            for i in ORDER:
                m[i] = _nt(_up(s1_v[i * 128 + rr * R1 // 2:i * 128 + (rr + 1) * R1 // 2, :]),
                           _up(tb1_v[i * 64:(i + 1) * 64, :]))
            c11, c12, c21, c22 = _comb(m)
            bu_v[4, rr * R1:(rr + 1) * R1, :] = c11
            bu_v[5, rr * R1:(rr + 1) * R1, :] = c12
            bu_v[4, HB + rr * R1:HB + (rr + 1) * R1, :] = c21
            bu_v[5, HB + rr * R1:HB + (rr + 1) * R1, :] = c22
        for tt in range(4):
            v = _nt(_up(xp_v[64 * tt:64 * (tt + 1), :]), _up(tb6_v[...]))
            bu_v[6, 128 * tt:128 * (tt + 1), :] = v
            bu_v[7, 128 * tt:128 * (tt + 1), :] = pltpu.roll(v, 64, 1)

    def scan():
        def step(j, t, hr, hi, lr, li):
            br = bu_v[2 * j, pl.ds(t, 8, stride=TS), :]
            bi = bu_v[2 * j + 1, pl.ds(t, 8, stride=TS), :]
            return lr * hr - li * hi + br, lr * hi + li * hr + bi

        zero = jnp.zeros((8, 128), F32)
        row = lax.broadcasted_iota(jnp.int32, (8, 128), 0)
        ends = []
        dep = None
        for j in range(4):
            er = ei = zero if dep is None else _after(zero, dep)
            lr, li = prm(0, j, 0), prm(0, j, 1)
            for t in range(TS):
                er, ei = step(j, t, er, ei, lr, li)
            ends.append((er, ei))
            dep = ei
        starts = []
        for j in range(4):
            er, ei = ends[j]
            xr = jnp.where(row == 0, jnp.broadcast_to(carry_v[2 * j:2 * j + 1, :], (8, 128)), pltpu.roll(er, 1, 0))
            xi = jnp.where(row == 0, jnp.broadcast_to(carry_v[2 * j + 1:2 * j + 2, :], (8, 128)), pltpu.roll(ei, 1, 0))
            for k, sh in enumerate([1, 2, 4]):
                ar, ai = prm(1 + k, j, 0), prm(1 + k, j, 1)
                yr = jnp.where(row >= sh, pltpu.roll(xr, sh, 0), 0.0)
                yi = jnp.where(row >= sh, pltpu.roll(xi, sh, 0), 0.0)
                xr, xi = xr + (ar * yr - ai * yi), xi + (ar * yi + ai * yr)
            starts.append((xr, xi))
        for j in range(4):
            sr, si = _after(starts[j][0], dep), starts[j][1]
            lr, li = prm(0, j, 0), prm(0, j, 1)
            for t in range(TS):
                sr, si = step(j, t, sr, si, lr, li)
                if j < 3:
                    hs_v[2 * j, pl.ds(t, 8, stride=TS), :] = sr
                    hs_v[2 * j + 1, pl.ds(t, 8, stride=TS), :] = si
                else:
                    hs_v[6, pl.ds(t, 8, stride=TS), :] = sr
                if t == MB - 1 - 7 * TS:
                    carry_v[2 * j:2 * j + 1, :] = sr[7:8, :]
                    carry_v[2 * j + 1:2 * j + 2, :] = si[7:8, :]
            dep = sr

    def h_operands():
        for q in range(2):
            m1 = slice(128 * q, 128 * (q + 1))
            m2 = slice(HB + 128 * q, HB + 128 * (q + 1))
            for j in range(3):
                ops = _rhs(hs_v[2 * j, m1, :], hs_v[2 * j, m2, :], hs_v[2 * j + 1, m1, :], hs_v[2 * j + 1, m2, :])
                for i, o in enumerate(ops):
                    uc_v[i * 128 + 64 * q:i * 128 + 64 * (q + 1), 128 * j:128 * (j + 1)] = _pk(o.astype(BF))
        for tt in range(4):
            uc_v[64 * tt:64 * (tt + 1), 384:512] = _pk(hs_v[6, 128 * tt:128 * (tt + 1), :].astype(BF))

    def gates(b):
        for tt in range(4):
            xt = xt_v[:, cols(b * MB + 128 * tt, 128)].astype(F32)
            g_v[tt:tt + 1, :] = jax.nn.sigmoid(jnp.sum(xt * col_v[1], axis=0, keepdims=True))

    def ffn_stage2():
        for q in range(2):
            f = [None] * 7
            for i in ORDER:
                f[i] = _nt(_up(a2_v[i * 112:(i + 1) * 112, :]), _up(u2_v[i * 128 + 64 * q:i * 128 + 64 * (q + 1), :]))
            c11, c12, c21, c22 = _comb(f)
            yf_v[0:DH, 128 * q:128 * (q + 1)] = c11
            yf_v[0:DH, HB + 128 * q:HB + 128 * (q + 1)] = c12
            yf_v[DH:D, 128 * q:128 * (q + 1)] = c21
            yf_v[DH:D, HB + 128 * q:HB + 128 * (q + 1)] = c22

    def mix(b, tt, dh, ys):
        rs = slice(DH * dh, DH * (dh + 1))
        ts = slice(128 * tt, 128 * (tt + 1))
        g = g_v[tt:tt + 1, :]
        a = ys + xt_v[rs, cols(b * MB + 128 * tt, 128)].astype(F32) * col_v[0, rs, :]
        o_v[b, rs, ts] = g * a + (0.5 - 0.5 * g) * yf_v[rs, ts]
        ocp(b, tt, dh).start()

    def ssm_stage2(b):
        for q in range(2):
            t1, t2 = q, 2 + q
            p6a = _nt(_up(ac_v[0:224, 384:512]), _up(uc_v[64 * t1:64 * (t1 + 1), 384:512]))
            p6b = _nt(_up(ac_v[0:224, 384:512]), _up(uc_v[64 * t2:64 * (t2 + 1), 384:512]))
            m = [None] * 7
            for i in ORDER_OUT:
                m[i] = _nt(_up(ac_v[i * 112:(i + 1) * 112, 0:384]),
                           _up(uc_v[i * 128 + 64 * q:i * 128 + 64 * (q + 1), 0:384]))
            s11, s12, s21, s22 = _comb(m)
            mix(b, t2, 0, s12 + p6b[0:DH])
            mix(b, t1, 1, s21 + p6a[DH:D])
            mix(b, t2, 1, s22 + p6b[DH:D])
            mix(b, t1, 0, s11 + p6a[0:DH])

    def wait_w(chunks):
        for c in chunks:
            for cp in wcp(c):
                cp.wait()

    xcp(0).wait()
    for cp in small:
        cp.wait()
    prep_x(0)
    wait_w([0])
    prep_w1(0)
    ffn_stage1([0])
    wait_w([1, 2])
    for c in (1, 2):
        prep_w1(c)
        ffn_stage1([c])
    params()
    wait_w([3, 4, 5, 6])
    for c in (3, 4, 5, 6):
        prep_w1(c)
        ffn_stage1([c])
    dcp.wait()
    for cp in bcp:
        cp.wait()
    prep_b()
    ssm_stage1()
    for cp in ccp:
        cp.wait()
    for b in range(1, NB):
        xcp(b).wait()
    prep_w2()
    prep_c()

    def second_half(b, nxt):
        ffn_stage2()
        scan()
        h_operands()
        gates(b)
        prep_x(nxt)
        ssm_stage2(b)

    second_half(0, 1)

    def block(b, c):
        ffn_stage1(range(NC))
        ssm_stage1()
        second_half(b, jnp.where(b + 1 < NB, b + 1, 0))
        return c

    lax.fori_loop(1, NB, block, 0)

    for b in range(NB):
        for tt in range(4):
            for dh in range(2):
                ocp(b, tt, dh).wait()


@jax.jit
def pallas_gated_mix__ssm_conv_s5__glu_gated_geglu__prompt_kernel(
    A_x: jax.Array,
    A_Lambda_re: jax.Array,
    A_Lambda_im: jax.Array,
    A_B_re: jax.Array,
    A_B_im: jax.Array,
    A_C_re: jax.Array,
    A_C_im: jax.Array,
    A_log_dt: jax.Array,
    A_Dskip: jax.Array,
    B_x: jax.Array,
    B_w_gate: jax.Array,
    B_w_up: jax.Array,
    B_w_down: jax.Array,
    gate_w: jax.Array,
):
    del B_x
    any_spec = pl.BlockSpec(memory_space=pl.ANY)
    V = pltpu.VMEM
    scratch = [V((D,), BF)] * 5 + [
        V((D, L), BF), V((D, D), BF), V((D, D), BF), V((D, D), BF), V((D, D), BF),
        V((D, FF), BF), V((D, FF), BF), V((D, FF), BF),
        V((7 * 128, KH), U32),
        V((25 * 64, 256), U32),
        V((MB // 2, 2 * KH), U32),
        V((49 * 64, FF // 2), U32),
        V((25 * 64, 256), U32),
        V((7 * 64, KH), U32),
        V((64, 2 * KH), U32),
        V((7 * 112, FF // 2), U32),
        V((7 * 112, 512), U32),
        V((7 * 128, FF // 2), U32),
        V((7 * 128, 512), U32),
        V((8, MB + 8, 128), F32),
        V((7, MB + 8, 128), F32),
        V((D, MB), F32),
        V((NB, D, MB), F32),
        V((32, 128), F32),
        V((2, D, 128), F32),
        V((8, 128), F32),
        V((8, D), F32),
        V((8, 128), F32),
    ] + [pltpu.SemaphoreType.DMA((n,)) for n in (5, NB, 2, 2, 2 * NC, 1, 8 * NB)]
    out = pl.pallas_call(
        _kernel,
        out_shape=jax.ShapeDtypeStruct((D, L), F32),
        in_specs=[any_spec] * 13,
        out_specs=any_spec,
        scratch_shapes=scratch,
        compiler_params=pltpu.CompilerParams(
            vmem_limit_bytes=100 * 1024 * 1024, disable_semaphore_checks=True, skip_device_barrier=True),
        name="gated_mix_s5_geglu",
    )(A_x.reshape(L, D).T, A_Lambda_re, A_Lambda_im, A_B_re, A_B_im, A_C_re, A_C_im, A_log_dt, A_Dskip,
      B_w_gate, B_w_up, B_w_down.T, gate_w)
    return out.T.reshape(1, L, D)
```

```python
import functools

import numpy as np
import jax
import jax.numpy as jnp
from jax import lax
import jax.experimental.pallas as pl
import jax.experimental.pallas.tpu as pltpu

BF = jnp.bfloat16
F32 = jnp.float32
U32 = jnp.uint32

L = 2048
D = 448
FF = 1792
MB = 512
NB = L // MB
HB = MB // 2
DH = D // 2
KH = 256
NC = FF // 256
TS = 65
RF = 64
R1 = 64
ORDER = (3, 4, 6, 0, 2, 1, 5)
ORDER_OUT = (2, 4, 1, 3, 0, 5, 6)
_C1 = float(np.sqrt(2.0 / np.pi))
_C2 = float(np.sqrt(2.0 / np.pi) * 0.044715)


def _pk(v):
    return pltpu.bitcast(v, U32)


def _up(v):
    return pltpu.bitcast(v, BF)


def _nn(a, b):
    return jnp.dot(a, b, preferred_element_type=F32)


def _nt(a, b):
    return lax.dot_general(a, b, (((1,), (1,)), ((), ())), preferred_element_type=F32)


def _lhs(a11, a12, a21, a22):
    return [a11 + a22, a21 + a22, a11, a22, a11 + a12, a21 - a11, a12 - a22]


def _rhs(b11, b12, b21, b22):
    return [b11 + b22, b11, b12 - b22, b21 - b11, b22, b11 + b12, b21 + b22]


def _comb(m):
    m1, m2, m3, m4, m5, m6, m7 = m
    return (m1 + m4 - m5 + m7, m3 + m5, m2 + m4, m1 - m2 + m3 + m6)


def _one_level(ops, a, b, c, d):
    raw = (a, b, c, d)
    out = []
    for v in ops(*[x.astype(F32) for x in raw]):
        out.append(v.astype(BF))
    plain = {2: 0, 3: 3} if ops is _lhs else {1: 0, 4: 3}
    for i, k in plain.items():
        out[i] = raw[k]
    return out


def _two_level(ops, blk):
    lvl1 = []
    for i in range(7):
        lvl1.append([[None, None], [None, None]])
    for a in range(2):
        for v in range(2):
            o = ops(blk[a][v], blk[a][2 + v], blk[2 + a][v], blk[2 + a][2 + v])
            for i in range(7):
                lvl1[i][a][v] = o[i]
    return lvl1, [ops(g[0][0], g[0][1], g[1][0], g[1][1]) for g in lvl1]


def _gelu_mul2(g, u):
    return (g * u) * (1.0 + jnp.tanh(g * (_C1 + _C2 * (g * g))))


def _after(x, dep):
    z = (pltpu.bitcast(dep, U32) >> 31) >> 1
    return pltpu.bitcast(pltpu.bitcast(x, U32) | z, F32)


def _kernel(xt_hbm, lre_hbm, lim_hbm, bre_hbm, bim_hbm, cre_hbm, cim_hbm, ldt_hbm, dsk_hbm,
            wg_hbm, wu_hbm, wdt_hbm, gw_hbm,
            out_hbm,
            lre_v, lim_v, ldt_v, dsk_v, gw_v,
            xt_v, bre_v, bim_v, cre_v, cim_v, wg_v, wu_v, wdt_v,
            s1_v, s2_v, xp_v, t2_v, tb2_v, tb1_v, tb6_v, a2_v, ac_v, u2_v, uc_v,
            bu_v, hs_v, yf_v, o_v, prm_v, col_v, carry_v, crow_v, g_v, sc_v,
            sem_small, sem_x, sem_b, sem_c, sem_w, sem_d, sem_o):
    small = [pltpu.make_async_copy(h, v, sem_small.at[i]) for i, (h, v) in enumerate(
        [(lre_hbm, lre_v), (lim_hbm, lim_v), (ldt_hbm, ldt_v), (dsk_hbm, dsk_v), (gw_hbm, gw_v)])]
    dcp = pltpu.make_async_copy(wdt_hbm, wdt_v, sem_d.at[0])
    bcp = [pltpu.make_async_copy(bre_hbm, bre_v, sem_b.at[0]), pltpu.make_async_copy(bim_hbm, bim_v, sem_b.at[1])]
    ccp = [pltpu.make_async_copy(cre_hbm, cre_v, sem_c.at[0]), pltpu.make_async_copy(cim_hbm, cim_v, sem_c.at[1])]

    def cols(start, size):
        if isinstance(start, int):
            return slice(start, start + size)
        return pl.ds(pl.multiple_of(start, 128), size)

    def xcp(b):
        return pltpu.make_async_copy(xt_hbm.at[:, cols(b * MB, MB)], xt_v.at[:, cols(b * MB, MB)], sem_x.at[b])

    def wcp(c):
        return [pltpu.make_async_copy(h.at[:, cols(c * 256, 256)], v.at[:, cols(c * 256, 256)], sem_w.at[2 * c + i])
                for i, (h, v) in enumerate([(wg_hbm, wg_v), (wu_hbm, wu_v)])]

    def ocp(b, tt, dh):
        rs = slice(DH * dh, DH * (dh + 1))
        return pltpu.make_async_copy(o_v.at[b, rs, 128 * tt:128 * (tt + 1)],
                                     out_hbm.at[rs, cols(b * MB + 128 * tt, 128)], sem_o.at[b * 8 + 2 * tt + dh])

    def start_in_order(lo, hi, fn):
        def body(i, c):
            fn(i)
            return c
        lax.fori_loop(lo, hi, body, 0)

    def start_w(c):
        for cp in wcp(c):
            cp.start()

    def start_rest(k):
        for n, group in enumerate([[dcp], bcp, ccp]):
            @pl.when(k == n)
            def _():
                for cp in group:
                    cp.start()

    xcp(0).start()
    for cp in small:
        cp.start()
    start_in_order(0, NC, start_w)
    start_in_order(0, 3, start_rest)
    start_in_order(1, NB, lambda b: xcp(b).start())

    bu_v[:, MB:MB + 8, :] = jnp.zeros((8, 8, 128), F32)

    def params():
        lre = lre_v[...].astype(F32)[None, :]
        lim = lim_v[...].astype(F32)[None, :]
        dt = jnp.exp(ldt_v[...].astype(F32)[None, :]).astype(BF).astype(F32)
        ea = jnp.exp(dt * lre)
        lbr = ea * jnp.cos(dt * lim)
        lbi = ea * jnp.sin(dt * lim)
        den = lre * lre + lim * lim
        nr = lbr - 1.0
        crow_v[0:1, :] = (nr * lre + lbi * lim) / den
        crow_v[1:2, :] = (lbi * lre - nr * lim) / den
        pr, pi = lbr, lbi
        for _ in range(6):
            pr, pi = pr * pr - pi * pi, 2.0 * pr * pi
        p1r, p1i = pr * lbr - pi * lbi, pr * lbi + pi * lbr
        p2r, p2i = p1r * p1r - p1i * p1i, 2.0 * p1r * p1i
        p4r, p4i = p2r * p2r - p2i * p2i, 2.0 * p2r * p2i
        for k, (vr, vi) in enumerate([(lbr, lbi), (p1r, p1i), (p2r, p2i), (p4r, p4i)]):
            for j in range(4):
                if j < 3:
                    tr, ti = vr[:, 128 * j:128 * (j + 1)], vi[:, 128 * j:128 * (j + 1)]
                else:
                    hr, hi = vr[:, 384:448], vi[:, 384:448]
                    tr, ti = jnp.concatenate([hr, hr], axis=1), jnp.concatenate([hi, -hi], axis=1)
                prm_v[8 * k + 2 * j:8 * k + 2 * j + 1, :] = tr
                prm_v[8 * k + 2 * j + 1:8 * k + 2 * j + 2, :] = ti
        col_v[0] = jnp.broadcast_to(dsk_v[...].astype(F32)[None, :], (128, D)).T
        col_v[1] = jnp.broadcast_to(gw_v[...].astype(F32)[None, :], (128, D)).T
        carry_v[...] = jnp.zeros((8, 128), F32)

    def prm(k, j, im):
        r = 8 * k + 2 * j + im
        return jnp.broadcast_to(prm_v[r:r + 1, :], (8, 128))

    def slot2(n):
        return (n // 2) * 64, slice((n % 2) * 128, (n % 2 + 1) * 128)

    def prep_x(b):
        zrow = jnp.zeros((2 * KH - D, 128), BF)
        xs = []
        for tt in range(4):
            x = jnp.concatenate([xt_v[:, cols(b * MB + 128 * tt, 128)], zrow], axis=0).T
            xp_v[64 * tt:64 * (tt + 1), :] = _pk(x)
            xs.append(x)
        lvl1, lvl2 = _two_level(_lhs, [[xs[r][:, 128 * k:128 * (k + 1)].astype(F32) for k in range(4)]
                                       for r in range(4)])
        for i in range(7):
            for a in range(2):
                if i == 2:
                    o = xs[a][:, 0:KH]
                elif i == 3:
                    o = xs[2 + a][:, KH:2 * KH]
                else:
                    o = jnp.concatenate(lvl1[i][a], axis=1).astype(BF)
                s1_v[i * 128 + 64 * a:i * 128 + 64 * (a + 1), :] = _pk(o)
            for j in range(7):
                r, lanes = slot2(7 * i + j)
                s2_v[r:r + 64, lanes] = _pk(lvl2[i][j].astype(BF))

    def prep_w1(c):
        zpad = jnp.zeros((2 * KH - D, 128), F32)
        blk = [[None] * 4 for _ in range(4)]
        for q, ref in enumerate((wg_v, wu_v)):
            w = ref[:, 256 * c:256 * (c + 1)].astype(F32)
            e = pltpu.bitcast(jnp.max(jnp.abs(w), axis=0, keepdims=True), jnp.int32) >> 23
            e = jnp.where(e == 0, 127, jnp.minimum(e, 253))
            sc_v[q:q + 1, 256 * c:256 * (c + 1)] = pltpu.bitcast(e << 23, F32)
            w = w * pltpu.bitcast((254 - e) << 23, F32)
            for nu in range(2):
                for k in range(4):
                    t = w[128 * k:min(128 * (k + 1), D), 128 * nu:128 * (nu + 1)]
                    blk[k][2 * q + nu] = t if k < 3 else jnp.concatenate([t, zpad], axis=0)
        _, lvl2 = _two_level(_rhs, blk)
        for n in range(49):
            t2_v[n * 64:(n + 1) * 64, 128 * c:128 * (c + 1)] = _pk(lvl2[n // 7][n % 7].astype(BF))

    def prep_b():
        zpad = jnp.zeros((128, 2 * KH - D), BF)

        def k2(ref, r0, n):
            return jnp.concatenate([ref[r0:r0 + n, KH:D], zpad[0:n]], axis=1)
        blk = [[None] * 4 for _ in range(4)]
        for q, ref in enumerate((bre_v, bim_v)):
            for nu in range(2):
                w = jnp.concatenate([ref[128 * nu:128 * (nu + 1), :].astype(F32), zpad.astype(F32)], axis=1)
                for k in range(4):
                    blk[k][2 * q + nu] = w[:, 128 * k:128 * (k + 1)]
        _, lvl2 = _two_level(_rhs, blk)
        for n in range(49):
            r, lanes = slot2(n)
            tb2_v[r:r + 64, lanes] = _pk(lvl2[n // 7][n % 7].astype(BF))
        ops = _one_level(_rhs, bre_v[256:384, 0:KH], bim_v[256:384, 0:KH], k2(bre_v, 256, 128), k2(bim_v, 256, 128))
        for i, o in enumerate(ops):
            tb1_v[i * 64:(i + 1) * 64, :] = _pk(o)
        tb6_v[0:32, 0:KH] = _pk(bre_v[384:448, 0:KH])
        tb6_v[32:64, 0:KH] = _pk(bim_v[384:448, 0:KH])
        tb6_v[0:32, KH:2 * KH] = _pk(k2(bre_v, 384, 64))
        tb6_v[32:64, KH:2 * KH] = _pk(k2(bim_v, 384, 64))

    def prep_w2():
        for c in range(NC):
            e = slice(256 * c, 256 * c + 128)
            o = slice(256 * c + 128, 256 * c + 256)
            we = wdt_v[:, e].astype(F32) * sc_v[1:2, e]
            wo = wdt_v[:, o].astype(F32) * sc_v[1:2, o]
            for i, v in enumerate(_lhs(we[0:DH], wo[0:DH], we[DH:D], wo[DH:D])):
                a2_v[i * 112:(i + 1) * 112, 128 * c:128 * (c + 1)] = _pk(v.astype(BF))

    def prep_c():
        cr = 2.0 * crow_v[0:1, :]
        ci = 2.0 * crow_v[1:2, :]
        parts = []
        for hf in range(2):
            cre = cre_v[DH * hf:DH * (hf + 1), :].astype(F32)
            cim = cim_v[DH * hf:DH * (hf + 1), :].astype(F32)
            are = cre * cr - cim * ci
            aim = -(cre * ci + cim * cr)
            ac_v[112 * hf:112 * (hf + 1), 384:512] = _pk(
                jnp.concatenate([are[:, 384:448], aim[:, 384:448]], axis=1).astype(BF))
            parts.append((are, aim))
        for j in range(3):
            cs = slice(128 * j, 128 * (j + 1))
            ops = _lhs(parts[0][0][:, cs], parts[0][1][:, cs], parts[1][0][:, cs], parts[1][1][:, cs])
            for i, v in enumerate(ops):
                ac_v[i * 112:(i + 1) * 112, cs] = _pk(v.astype(BF))

    def two_level_products(r0, rows, dot, rhs):
        outer = [None] * 7
        for i in ORDER:
            p = [None] * 7
            for j in ORDER:
                r, lanes = slot2(7 * i + j)
                p[j] = dot(_up(s2_v[r + r0 // 2:r + (r0 + rows) // 2, lanes]), _up(rhs(7 * i + j)))
            outer[i] = _comb(p)
        out = {}
        for a in range(2):
            for nu in range(2):
                c = _comb([outer[i][2 * a + nu] for i in range(7)])
                for p in range(2):
                    for q in range(2):
                        out[(2 * p + a, q, nu)] = c[2 * p + q]
        return out

    def ffn_stage1(chunks):
        for c in chunks:
            for rr in range(128 // RF):
                z = two_level_products(rr * RF, RF, _nn, lambda n: t2_v[n * 64:(n + 1) * 64, 128 * c:128 * (c + 1)])
                sg = [sc_v[0:1, 256 * c + 128 * nu:256 * c + 128 * (nu + 1)] for nu in range(2)]
                hh = {(tt, nu): _gelu_mul2(z[(tt, 0, nu)] * sg[nu], z[(tt, 1, nu)])
                      for tt in range(4) for nu in range(2)}
                for a in range(2):
                    ops = _rhs(hh[(a, 0)], hh[(2 + a, 0)], hh[(a, 1)], hh[(2 + a, 1)])
                    for i, o in enumerate(ops):
                        r = i * 128 + 64 * a + rr * RF // 2
                        u2_v[r:r + RF // 2, 128 * c:128 * (c + 1)] = _pk(o.astype(BF))

    def ssm_stage1():
        def rhs(n):
            r, lanes = slot2(n)
            return tb2_v[r:r + 64, lanes]
        z = two_level_products(0, 128, _nt, rhs)
        for (tt, q, nu), v in z.items():
            bu_v[2 * nu + q, 128 * tt:128 * (tt + 1), :] = v
        for rr in range(HB // R1):
            m = [None] * 7
            for i in ORDER:
                m[i] = _nt(_up(s1_v[i * 128 + rr * R1 // 2:i * 128 + (rr + 1) * R1 // 2, :]),
                           _up(tb1_v[i * 64:(i + 1) * 64, :]))
            c11, c12, c21, c22 = _comb(m)
            bu_v[4, rr * R1:(rr + 1) * R1, :] = c11
            bu_v[5, rr * R1:(rr + 1) * R1, :] = c12
            bu_v[4, HB + rr * R1:HB + (rr + 1) * R1, :] = c21
            bu_v[5, HB + rr * R1:HB + (rr + 1) * R1, :] = c22
        for tt in range(4):
            v = _nt(_up(xp_v[64 * tt:64 * (tt + 1), :]), _up(tb6_v[...]))
            bu_v[6, 128 * tt:128 * (tt + 1), :] = v
            bu_v[7, 128 * tt:128 * (tt + 1), :] = pltpu.roll(v, 64, 1)

    def scan():
        def step(j, t, hr, hi, lr, li):
            br = bu_v[2 * j, pl.ds(t, 8, stride=TS), :]
            bi = bu_v[2 * j + 1, pl.ds(t, 8, stride=TS), :]
            return lr * hr - li * hi + br, lr * hi + li * hr + bi

        zero = jnp.zeros((8, 128), F32)
        row = lax.broadcasted_iota(jnp.int32, (8, 128), 0)
        ends = []
        dep = None
        for j in range(4):
            er = ei = zero if dep is None else _after(zero, dep)
            lr, li = prm(0, j, 0), prm(0, j, 1)
            for t in range(TS):
                er, ei = step(j, t, er, ei, lr, li)
            ends.append((er, ei))
            dep = ei
        starts = []
        for j in range(4):
            er, ei = ends[j]
            xr = jnp.where(row == 0, jnp.broadcast_to(carry_v[2 * j:2 * j + 1, :], (8, 128)), pltpu.roll(er, 1, 0))
            xi = jnp.where(row == 0, jnp.broadcast_to(carry_v[2 * j + 1:2 * j + 2, :], (8, 128)), pltpu.roll(ei, 1, 0))
            for k, sh in enumerate([1, 2, 4]):
                ar, ai = prm(1 + k, j, 0), prm(1 + k, j, 1)
                yr = jnp.where(row >= sh, pltpu.roll(xr, sh, 0), 0.0)
                yi = jnp.where(row >= sh, pltpu.roll(xi, sh, 0), 0.0)
                xr, xi = xr + (ar * yr - ai * yi), xi + (ar * yi + ai * yr)
            starts.append((xr, xi))
        for j in range(4):
            sr, si = _after(starts[j][0], dep), starts[j][1]
            lr, li = prm(0, j, 0), prm(0, j, 1)
            for t in range(TS):
                sr, si = step(j, t, sr, si, lr, li)
                if j < 3:
                    hs_v[2 * j, pl.ds(t, 8, stride=TS), :] = sr
                    hs_v[2 * j + 1, pl.ds(t, 8, stride=TS), :] = si
                else:
                    hs_v[6, pl.ds(t, 8, stride=TS), :] = sr
                if t == MB - 1 - 7 * TS:
                    carry_v[2 * j:2 * j + 1, :] = sr[7:8, :]
                    carry_v[2 * j + 1:2 * j + 2, :] = si[7:8, :]
            dep = sr

    def h_operands():
        for q in range(2):
            m1 = slice(128 * q, 128 * (q + 1))
            m2 = slice(HB + 128 * q, HB + 128 * (q + 1))
            for j in range(3):
                ops = _rhs(hs_v[2 * j, m1, :], hs_v[2 * j, m2, :], hs_v[2 * j + 1, m1, :], hs_v[2 * j + 1, m2, :])
                for i, o in enumerate(ops):
                    uc_v[i * 128 + 64 * q:i * 128 + 64 * (q + 1), 128 * j:128 * (j + 1)] = _pk(o.astype(BF))
        for tt in range(4):
            uc_v[64 * tt:64 * (tt + 1), 384:512] = _pk(hs_v[6, 128 * tt:128 * (tt + 1), :].astype(BF))

    def gates(b):
        for tt in range(4):
            xt = xt_v[:, cols(b * MB + 128 * tt, 128)].astype(F32)
            g_v[tt:tt + 1, :] = jax.nn.sigmoid(jnp.sum(xt * col_v[1], axis=0, keepdims=True))

    def ffn_stage2():
        for q in range(2):
            f = [None] * 7
            for i in ORDER:
                f[i] = _nt(_up(a2_v[i * 112:(i + 1) * 112, :]), _up(u2_v[i * 128 + 64 * q:i * 128 + 64 * (q + 1), :]))
            c11, c12, c21, c22 = _comb(f)
            yf_v[0:DH, 128 * q:128 * (q + 1)] = c11
            yf_v[0:DH, HB + 128 * q:HB + 128 * (q + 1)] = c12
            yf_v[DH:D, 128 * q:128 * (q + 1)] = c21
            yf_v[DH:D, HB + 128 * q:HB + 128 * (q + 1)] = c22

    def mix(b, tt, dh, ys):
        rs = slice(DH * dh, DH * (dh + 1))
        ts = slice(128 * tt, 128 * (tt + 1))
        g = g_v[tt:tt + 1, :]
        a = ys + xt_v[rs, cols(b * MB + 128 * tt, 128)].astype(F32) * col_v[0, rs, :]
        o_v[b, rs, ts] = g * a + (0.5 - 0.5 * g) * yf_v[rs, ts]
        ocp(b, tt, dh).start()

    def ssm_stage2(b):
        for q in range(2):
            t1, t2 = q, 2 + q
            p6a = _nt(_up(ac_v[0:224, 384:512]), _up(uc_v[64 * t1:64 * (t1 + 1), 384:512]))
            p6b = _nt(_up(ac_v[0:224, 384:512]), _up(uc_v[64 * t2:64 * (t2 + 1), 384:512]))
            m = [None] * 7
            for i in ORDER_OUT:
                m[i] = _nt(_up(ac_v[i * 112:(i + 1) * 112, 0:384]),
                           _up(uc_v[i * 128 + 64 * q:i * 128 + 64 * (q + 1), 0:384]))
            s11, s12, s21, s22 = _comb(m)
            mix(b, t2, 0, s12 + p6b[0:DH])
            mix(b, t1, 1, s21 + p6a[DH:D])
            mix(b, t2, 1, s22 + p6b[DH:D])
            mix(b, t1, 0, s11 + p6a[0:DH])

    def wait_w(chunks):
        for c in chunks:
            for cp in wcp(c):
                cp.wait()

    xcp(0).wait()
    for cp in small:
        cp.wait()
    prep_x(0)
    wait_w([0])
    prep_w1(0)
    ffn_stage1([0])
    wait_w([1, 2])
    for c in (1, 2):
        prep_w1(c)
        ffn_stage1([c])
    params()
    wait_w([3, 4, 5, 6])
    for c in (3, 4, 5, 6):
        prep_w1(c)
        ffn_stage1([c])
    dcp.wait()
    for cp in bcp:
        cp.wait()
    prep_b()
    ssm_stage1()
    for cp in ccp:
        cp.wait()
    for b in range(1, NB):
        xcp(b).wait()
    prep_w2()
    prep_c()

    def second_half(b, nxt):
        ffn_stage2()
        scan()
        h_operands()
        gates(b)
        prep_x(nxt)
        ssm_stage2(b)

    second_half(0, 1)

    def block(b, c):
        ffn_stage1(range(NC))
        ssm_stage1()
        second_half(b, jnp.where(b + 1 < NB, b + 1, 0))
        return c

    lax.fori_loop(1, NB, block, 0)

    for b in range(NB):
        for tt in range(4):
            for dh in range(2):
                ocp(b, tt, dh).wait()


@jax.jit
def pallas_gated_mix__ssm_conv_s5__glu_gated_geglu__prompt_kernel(
    A_x: jax.Array,
    A_Lambda_re: jax.Array,
    A_Lambda_im: jax.Array,
    A_B_re: jax.Array,
    A_B_im: jax.Array,
    A_C_re: jax.Array,
    A_C_im: jax.Array,
    A_log_dt: jax.Array,
    A_Dskip: jax.Array,
    B_x: jax.Array,
    B_w_gate: jax.Array,
    B_w_up: jax.Array,
    B_w_down: jax.Array,
    gate_w: jax.Array,
):
    del B_x
    any_spec = pl.BlockSpec(memory_space=pl.ANY)
    V = pltpu.VMEM
    scratch = [V((D,), BF)] * 5 + [
        V((D, L), BF), V((D, D), BF), V((D, D), BF), V((D, D), BF), V((D, D), BF),
        V((D, FF), BF), V((D, FF), BF), V((D, FF), BF),
        V((7 * 128, KH), U32),
        V((25 * 64, 256), U32),
        V((MB // 2, 2 * KH), U32),
        V((49 * 64, FF // 2), U32),
        V((25 * 64, 256), U32),
        V((7 * 64, KH), U32),
        V((64, 2 * KH), U32),
        V((7 * 112, FF // 2), U32),
        V((7 * 112, 512), U32),
        V((7 * 128, FF // 2), U32),
        V((7 * 128, 512), U32),
        V((8, MB + 8, 128), F32),
        V((7, MB + 8, 128), F32),
        V((D, MB), F32),
        V((NB, D, MB), F32),
        V((32, 128), F32),
        V((2, D, 128), F32),
        V((8, 128), F32),
        V((8, D), F32),
        V((8, 128), F32),
        V((8, FF), F32),
    ] + [pltpu.SemaphoreType.DMA((n,)) for n in (5, NB, 2, 2, 2 * NC, 1, 8 * NB)]
    out = pl.pallas_call(
        _kernel,
        out_shape=jax.ShapeDtypeStruct((D, L), F32),
        in_specs=[any_spec] * 13,
        out_specs=any_spec,
        scratch_shapes=scratch,
        compiler_params=pltpu.CompilerParams(
            vmem_limit_bytes=100 * 1024 * 1024, disable_semaphore_checks=True, skip_device_barrier=True),
        name="gated_mix_s5_geglu",
    )(A_x.reshape(L, D).T, A_Lambda_re, A_Lambda_im, A_B_re, A_B_im, A_C_re, A_C_im, A_log_dt, A_Dskip,
      B_w_gate, B_w_up, B_w_down.T, gate_w)
    return out.T.reshape(1, L, D)
```
